```python
import os as _os
_os.environ.setdefault("JAX_PLATFORMS", "cpu")
import jax
import jax.numpy as jnp

def _softmax(x, axis=-1):
    return jax.nn.softmax(x, axis=axis)
def _gelu(x):
    return jax.nn.gelu(x, approximate=True)
def _silu(x):
    return jax.nn.silu(x)
def _sigmoid(x):
    return jax.nn.sigmoid(x)
def _layernorm(x, axis=-1, eps=1e-5):
    m = jnp.mean(x, axis=axis, keepdims=True)
    v = jnp.var(x, axis=axis, keepdims=True)
    return (x - m) / jnp.sqrt(v + eps)
def _scatter_add(tgt, idx, src, axis=0):
    return tgt.at[idx].add(src)
def _segment_sum(src, seg, n):
    return jax.ops.segment_sum(src, seg, n)
class _Rng:
    def __init__(self, key):
        self._k = key
    def _next(self):
        self._k, sub = jax.random.split(self._k)
        return sub
    def normal(self, shape):
        return jax.random.normal(self._next(), shape, dtype=jnp.bfloat16)
    def randint(self, lo, hi, shape):
        return jax.random.randint(self._next(), shape, lo, hi, dtype=jnp.int32)
    def uniform(self, shape, lo=0.0, hi=1.0):
        return jax.random.uniform(self._next(), shape, jnp.bfloat16, lo, hi)
    def permutation(self, n):
        return jax.random.permutation(self._next(), n)


kernel_name = 'interleave_layers__mha_block__dense_activation_gelu__prompt'

def setup_inputs():
    _rng = _Rng(jax.random.key(int.from_bytes(__import__("os").urandom(4), "little")))
    _w = (lambda a: (lambda t: t.astype(jnp.bfloat16) if jnp.issubdtype(t.dtype, jnp.floating) else t)(jnp.asarray(a)))
    def _A_setup():
        B, S, D, H = 1, 2048, 512, 32
        return {
            "x": _w((lambda *s: _rng.normal(s) * 0.05)(B, S, D)),
            "wqkv": _w((lambda *s: _rng.normal(s) * 0.05)(D, 3 * D)),
            "wo": _w((lambda *s: _rng.normal(s) * 0.05)(D, D)),
        }
    _A_in = _A_setup()

    def _B_setup():
        B, S, D, F = 1, 2048, 512, 1792
        return {
            "x": _w((lambda *s: _rng.normal(s) * 0.05)(B, S, D)),
            "w1": _w((lambda *s: _rng.normal(s) * 0.4)(D, F) * (D ** -0.5)),
            "b1": _w((lambda *s: _rng.normal(s) * 0.4)(F) * 0.01),
            "w2": _w((lambda *s: _rng.normal(s) * 0.4)(F, D) * (F ** -0.5)),
            "b2": _w((lambda *s: _rng.normal(s) * 0.4)(D) * 0.01),
        }
    _B_in = _B_setup()

    return {
        "A_x": _A_in["x"],
        "A_wqkv": _A_in["wqkv"],
        "A_wo": _A_in["wo"],
        "B_x": _B_in["x"],
        "B_w1": _B_in["w1"],
        "B_b1": _B_in["b1"],
        "B_w2": _B_in["w2"],
        "B_b2": _B_in["b2"],
    }

def reference(A_x, A_wqkv, A_wo, B_x, B_w1, B_b1, B_w2, B_b2):
    def _A_ref(x, wqkv, wo):
        B, S, D = x.shape
        H = 32
        Dh = D // H
        qkv = (lambda x, *d: x.transpose(*d))((x @ wqkv).reshape(B, S, 3, H, Dh), 2, 0, 3, 1, 4)
        q, k, v = qkv[0], qkv[1], qkv[2]
        scores = jnp.einsum("bhqd,bhkd->bhqk", q, k) * (Dh ** -0.5)
        p = _softmax(scores, axis=-1)
        o = jnp.einsum("bhqk,bhkd->bhqd", p, v)
        return (lambda x, *d: x.transpose(*d))(o, 0, 2, 1, 3).reshape(B, S, D) @ wo

    def _B_ref(x, w1, b1, w2, b2):
        h = jnp.einsum("bsd,df->bsf", x, w1) + b1
        h = _gelu(h)
        return jnp.einsum("bsf,fd->bsd", h, w2) + b2

    x = A_x
    x = x + _A_ref(_layernorm(x, axis=-1), A_wqkv, A_wo)
    x = x + _B_ref(_layernorm(x, axis=-1), B_w1, B_b1, B_w2, B_b2)
    x = x + _A_ref(_layernorm(x, axis=-1), A_wqkv, A_wo)
    x = x + _B_ref(_layernorm(x, axis=-1), B_w1, B_b1, B_w2, B_b2)
    return x
```

```python
import math

import jax
import jax.numpy as jnp
from jax import lax
import jax.experimental.pallas as pl
import jax.experimental.pallas.tpu as pltpu

F32 = jnp.float32
BF16 = jnp.bfloat16

N_HEADS = 32
LN_EPS = 1e-5
TQ = 512
CK = 128
NSUB = 4
TM = 256


def _layernorm(x):
    m = jnp.mean(x, axis=-1, keepdims=True)
    xc = x - m
    v = jnp.mean(xc * xc, axis=-1, keepdims=True)
    return xc * lax.rsqrt(v + LN_EPS)


def _gelu_tanh(x):
    c = math.sqrt(2.0 / math.pi)
    return 0.5 * x * (1.0 + jnp.tanh(c * (x + 0.044715 * (x * x * x))))


def _make_kernel(S, D, F):
    H = N_HEADS
    DH = D // H
    HPG = 128 // DH
    nq = S // TQ
    nunits = H * nq
    ngroups = nunits // NSUB
    nck = S // CK
    nt = S // TM
    qscale = (DH ** -0.5) * math.log2(math.e)

    def kernel(x_in, wqkv, wo, w1, b1, w2, b2, out,
               x, wqvt, qt, k, vt, ot, s0, s1, m0, m1):

        def qkv_tile(rows, xt):
            xn = _layernorm(xt).astype(BF16)
            k[rows, :] = jnp.dot(xn, wqkv[:, D:2 * D],
                                 preferred_element_type=F32).astype(BF16)
            qv = lax.dot_general(wqvt[...], xn, (((1,), (1,)), ((), ())),
                                 preferred_element_type=F32)
            qt[:, rows] = (qv[:D] * qscale).astype(BF16)
            vt[:, rows] = qv[D:].astype(BF16)

        def wq(u):
            h = u // nq
            qi = u % nq
            g = h // HPG
            hh = h % HPG
            slab = qt[pl.ds(pl.multiple_of(g * 128, 128), 128),
                      pl.ds(pl.multiple_of(qi * TQ, TQ), TQ)]
            rows = lax.broadcasted_iota(jnp.int32, (128, TQ), 0)
            w = jnp.where((rows // DH) == hh, slab, jnp.zeros_like(slab))
            return w, g

        def a_chunk(w, g, c, sbuf, j, m):
            kc = k[pl.ds(c * CK, CK), pl.ds(pl.multiple_of(g * 128, 128), 128)]
            s = jnp.dot(kc, w, preferred_element_type=F32)
            sbuf[j, pl.ds(c * CK, CK), :] = s
            for r in range(CK // 8):
                sr = s[r * 8:(r + 1) * 8, :]
                m = sr if m is None else jnp.maximum(m, sr)
            return m

        def a_fin(ma, j, m):
            ma[j] = jnp.broadcast_to(jnp.max(m, axis=0, keepdims=True), (8, TQ))

        def b_chunk(u, c, sbuf, j, m, l, acc):
            h = u // nq
            s = sbuf[j, pl.ds(c * CK, CK), :]
            p = jnp.exp2(s.reshape(CK // 8, 8, TQ) - m[None]).reshape(CK, TQ)
            for r in reversed(range(CK // 8)):
                pr = p[r * 8:(r + 1) * 8, :]
                l = pr if l is None else l + pr
            vc = vt[pl.ds(pl.multiple_of(h * DH, DH), DH), pl.ds(c * CK, CK)]
            o = jnp.dot(vc, p.astype(BF16), preferred_element_type=F32)
            return l, (o if acc is None else acc + o)

        def b_fin(u, l, acc):
            h = u // nq
            qi = u % nq
            lsum = jnp.sum(l, axis=0, keepdims=True)
            ot[pl.ds(pl.multiple_of(h * DH, DH), DH),
               pl.ds(pl.multiple_of(qi * TQ, TQ), TQ)] = (acc / lsum).astype(BF16)

        def step(ga, sa, ma, gb, sb, mb):
            for j in range(NSUB):
                if ga is not None:
                    w, g = wq(ga * NSUB + j)
                if gb is not None:
                    mB = mb[j]
                m = l = acc = None
                for c in range(nck):
                    if ga is not None:
                        m = a_chunk(w, g, c, sa, j, m)
                    if gb is not None:
                        l, acc = b_chunk(gb * NSUB + j, c, sb, j, mB, l, acc)
                if ga is not None:
                    a_fin(ma, j, m)
                if gb is not None:
                    b_fin(gb * NSUB + j, l, acc)

        def attention():
            step(0, s0, m0, None, None, None)

            def body(i, carry):
                @pl.when(i % 2 == 0)
                def _():
                    step(i + 1, s1, m1, i, s0, m0)

                @pl.when(i % 2 == 1)
                def _():
                    step(i + 1, s0, m0, i, s1, m1)
                return carry
            lax.fori_loop(0, ngroups - 1, body, 0)
            last = ngroups - 1
            if last % 2 == 0:
                step(None, None, None, last, s0, m0)
            else:
                step(None, None, None, last, s1, m1)

        def post_tile(rows):
            attn = lax.dot_general(ot[:, rows], wo[...], (((0,), (0,)), ((), ())),
                                   preferred_element_type=F32)
            x1 = x[rows, :] + attn
            xn = _layernorm(x1).astype(BF16)
            hid = jnp.dot(xn, w1[...], preferred_element_type=F32) + b1[...].astype(F32)
            hid = _gelu_tanh(hid).astype(BF16)
            y = jnp.dot(hid, w2[...], preferred_element_type=F32) + b2[...].astype(F32)
            return x1 + y

        layer = pl.program_id(0)

        @pl.when(layer == 0)
        def _():
            wqvt[0:D, :] = wqkv[:, 0:D].astype(F32).T.astype(BF16)
            wqvt[D:2 * D, :] = wqkv[:, 2 * D:3 * D].astype(F32).T.astype(BF16)

            def body(t, carry):
                rows = pl.ds(pl.multiple_of(t * TM, TM), TM)
                xt = x_in[rows, :].astype(F32)
                x[rows, :] = xt
                qkv_tile(rows, xt)
                return carry
            lax.fori_loop(0, nt, body, 0)

        attention()

        @pl.when(layer == 0)
        def _():
            def body(t, carry):
                rows = pl.ds(pl.multiple_of(t * TM, TM), TM)
                x2 = post_tile(rows)
                x[rows, :] = x2
                qkv_tile(rows, x2)
                return carry
            lax.fori_loop(0, nt, body, 0)

        @pl.when(layer == 1)
        def _():
            def body(t, carry):
                rows = pl.ds(pl.multiple_of(t * TM, TM), TM)
                out[rows, :] = post_tile(rows).astype(out.dtype)
                return carry
            lax.fori_loop(0, nt, body, 0)

    return kernel


@jax.jit
def pallas_interleave_layers__mha_block__dense_activation_gelu__prompt_kernel(
    A_x: jax.Array,
    A_wqkv: jax.Array,
    A_wo: jax.Array,
    B_x: jax.Array,
    B_w1: jax.Array,
    B_b1: jax.Array,
    B_w2: jax.Array,
    B_b2: jax.Array,
):
    B, S, D = A_x.shape
    F = B_w1.shape[1]
    assert B == 1
    x2d = A_x.reshape(S, D)
    b1 = B_b1.reshape(1, F)
    b2 = B_b2.reshape(1, D)

    def full(shape):
        return pl.BlockSpec(shape, lambda i: (0,) * len(shape))

    out = pl.pallas_call(
        _make_kernel(S, D, F),
        grid=(2,),
        in_specs=[full((S, D)), full((D, 3 * D)), full((D, D)), full((D, F)),
                  full((1, F)), full((F, D)), full((1, D))],
        out_specs=full((S, D)),
        out_shape=jax.ShapeDtypeStruct((S, D), A_x.dtype),
        scratch_shapes=[
            pltpu.VMEM((S, D), F32),
            pltpu.VMEM((2 * D, D), BF16),
            pltpu.VMEM((D, S), BF16),
            pltpu.VMEM((S, D), BF16),
            pltpu.VMEM((D, S), BF16),
            pltpu.VMEM((D, S), BF16),
            pltpu.VMEM((NSUB, S, TQ), F32),
            pltpu.VMEM((NSUB, S, TQ), F32),
            pltpu.VMEM((NSUB, 8, TQ), F32),
            pltpu.VMEM((NSUB, 8, TQ), F32),
        ],
        compiler_params=pltpu.CompilerParams(
            dimension_semantics=("arbitrary",),
            vmem_limit_bytes=100 * 1024 * 1024,
        ),
    )(x2d, A_wqkv, A_wo, B_w1, b1, B_w2, b2)
    return out.reshape(B, S, D)
```

```python
import math

import jax
import jax.numpy as jnp
from jax import lax
import jax.experimental.pallas as pl
import jax.experimental.pallas.tpu as pltpu

F32 = jnp.float32
BF16 = jnp.bfloat16
U32 = jnp.uint32

N_HEADS = 32
LN_EPS = 1e-5
TQ = 512
CK = 128
TM = 256
TS = 128
VPU_CHUNKS = (0, 1, 2, 4, 5, 6, 8, 9, 10, 12, 13, 14)


def _layernorm(x):
    m = jnp.mean(x, axis=-1, keepdims=True)
    xc = x - m
    v = jnp.mean(xc * xc, axis=-1, keepdims=True)
    return xc * lax.rsqrt(v + LN_EPS)


def _gelu_tanh(x):
    c = math.sqrt(2.0 / math.pi)
    return 0.5 * x * (1.0 + jnp.tanh(c * (x + 0.044715 * (x * x * x))))


def _make_kernel(S, D, F):
    H = N_HEADS
    DH = D // H
    HPG = 128 // DH
    nq = S // TQ
    nck = S // CK
    nt = S // TM
    ntl = TQ // 128
    qscale = (DH ** -0.5) * math.log2(math.e)
    offl = list(VPU_CHUNKS)
    noff = len(offl)
    ngrp = (noff + 7) // 8
    nsteps = nq * nck
    pieces = [(i, r, t) for i in range(noff) for r in range(2) for t in range(ntl)]
    nrows = sum((CK - 16 if c in offl else CK) // 8 for c in range(nck))
    piece_pos = {}
    for n, p in enumerate(pieces):
        piece_pos.setdefault(int((n + 0.5) * nrows / len(pieces)), []).append(p)

    def kernel(x_hbm, wqkv_hbm, wo_hbm, w1_hbm, b1, w2_hbm, b2, out_hbm,
               x_in, wqkv, wo, w1, w2, out,
               x, wqvt, qt, k, vt, ot, s0, s1, m0, m1, qf, kb0, kb1, kr0, kr1, kto,
               xsem, wsem, osem):

        def x_copy(t):
            return pltpu.make_async_copy(x_hbm.at[pl.ds(t * TM, TM), :],
                                         x_in.at[pl.ds(t * TM, TM), :], xsem.at[t])

        def out_copy(t):
            return pltpu.make_async_copy(out.at[pl.ds(t * TM, TM), :],
                                         out_hbm.at[pl.ds(t * TM, TM), :], osem.at[t])

        wqkv_copy = pltpu.make_async_copy(wqkv_hbm, wqkv, wsem.at[0])
        late_copies = [pltpu.make_async_copy(wo_hbm, wo, wsem.at[1]),
                       pltpu.make_async_copy(w1_hbm, w1, wsem.at[2]),
                       pltpu.make_async_copy(w2_hbm, w2, wsem.at[3])]

        def qkv_mm(r0, xn):
            rows = pl.ds(r0, TS)
            kk = jnp.dot(xn, wqkv[:, D:2 * D], preferred_element_type=F32).astype(BF16)
            k[pl.ds(pl.multiple_of(r0 // 2, TS // 2), TS // 2), :] = pltpu.bitcast(kk, U32)
            qv = lax.dot_general(wqvt[...], xn, (((1,), (1,)), ((), ())),
                                 preferred_element_type=F32)
            qt[:, rows] = pltpu.bitcast((qv[:D] * qscale).astype(BF16), U32)
            vt[:, rows] = pltpu.bitcast(qv[D:].astype(BF16), U32)

        def subrows(t):
            return [pl.multiple_of(t * TM + i * TS, TS) for i in range(TM // TS)]

        def head_rows(h):
            return pl.ds(pl.multiple_of(h * (DH // 2), DH // 2), DH // 2)

        def prep(h, n, kb, kr):
            g = h // HPG
            hh = h % HPG
            nr = (S // 2) // nsteps
            kc = k[pl.ds(n * nr, nr), pl.ds(pl.multiple_of(g * 128, 128), 128)]
            kr[pl.ds(n * nr, nr), :] = pltpu.roll(kc, (128 - hh * DH) % 128, 1)
            per = nsteps // (DH * ngrp)
            if n % per == 0:
                gi, d = (n // per) // DH, (n // per) % DH
                nk = min(128, (noff - gi * 8) * 16)
                row = kto[gi, h, d:d + 1, :]
                kb[d, gi * 128:gi * 128 + nk, :] = jnp.broadcast_to(row, (128, 128)).T[:nk]

        def piece(p, kba, sbuf, j, m):
            i, r, t = p
            acc = None
            for d in range(DH):
                c0 = j * TQ + t * 128
                qb = jnp.broadcast_to(qf[d:d + 1, c0:c0 + 128], (8, 128))
                pr = kba[d, i * 16 + r * 8:i * 16 + (r + 1) * 8, :] * qb
                acc = pr if acc is None else acc + pr
            sbuf[j, pl.ds(offl[i] * CK + CK - 16 + r * 8, 8), t * 128:(t + 1) * 128] = acc
            m[t] = jnp.maximum(m[t], acc)

        def b_chunk(h, c, sbuf, j, m, l, acc):
            s = sbuf[j, pl.ds(c * CK, CK), :]
            p = jnp.exp2(s.reshape(CK // 8, 8, TQ) - m[None]).reshape(CK, TQ)
            for r in reversed(range(CK // 8)):
                pr = p[r * 8:(r + 1) * 8, :]
                l = pr if l is None else l + pr
            vc = pltpu.bitcast(vt[head_rows(h), pl.ds(c * CK, CK)], BF16)
            o = jnp.dot(vc, p.astype(BF16), preferred_element_type=F32)
            return l, (o if acc is None else o + acc)

        def b_fin(h, j, l, acc):
            lsum = jnp.sum(l, axis=0, keepdims=True)
            ot[pl.ds(pl.multiple_of(h * DH, DH), DH), pl.ds(j * TQ, TQ)] = (
                acc / lsum).astype(BF16)

        def step(ha, sa, ma, kba, kra, hb, sb, mb, hn, kbn, krn):
            use_vpu = kba is not None
            if ha is not None and use_vpu:
                qf[...] = pltpu.bitcast(qt[head_rows(ha), :], BF16).astype(F32)
            for j in range(nq):
                if ha is not None:
                    w = pltpu.bitcast(qt[head_rows(ha), pl.ds(j * TQ, TQ)], BF16)
                if hb is not None:
                    mB = mb[j]
                l = acc = None
                m = [None] * ntl
                rowpos = 0
                for c in range(nck):
                    if ha is not None:
                        nm = CK - 16 if (use_vpu and c in offl) else CK
                        kc = pltpu.bitcast(kra[pl.ds(c * CK // 2, nm // 2), 0:128], BF16)
                        s = jnp.dot(kc[:, 0:DH], w, preferred_element_type=F32)
                        sa[j, pl.ds(c * CK, nm), :] = s
                        for r in range(nm // 8):
                            for t in range(ntl):
                                sr = s[r * 8:(r + 1) * 8, t * 128:(t + 1) * 128]
                                m[t] = sr if m[t] is None else jnp.maximum(m[t], sr)
                            if use_vpu:
                                for p in piece_pos.get(rowpos, []):
                                    piece(p, kba, sa, j, m)
                            rowpos += 1
                    if hb is not None:
                        l, acc = b_chunk(hb, c, sb, j, mB, l, acc)
                    if hn is not None:
                        prep(hn, j * nck + c, kbn, krn)
                if ha is not None:
                    mm = jnp.concatenate(m, axis=1)
                    ma[j] = jnp.broadcast_to(jnp.max(mm, axis=0, keepdims=True), (8, TQ))
                if hb is not None:
                    b_fin(hb, j, l, acc)

        def attention():
            for gi in range(ngrp):
                cs = [offl[min(gi * 8 + e, noff - 1)] for e in range(8)]
                rows = jnp.concatenate(
                    [k[(c * CK + CK - 16) // 2:(c * CK + CK) // 2, :] for c in cs], axis=0)
                rows = pltpu.bitcast(rows, BF16).astype(F32)
                kto[gi] = rows.T.reshape(H, DH, 128)
            step(0, s0, m0, None, k, None, None, None, 1, kb1, kr1)

            def body(i, carry):
                nn = jnp.minimum(i + 2, H - 1)

                @pl.when(i % 2 == 0)
                def _():
                    step(i + 1, s1, m1, kb1, kr1, i, s0, m0, nn, kb0, kr0)

                @pl.when(i % 2 == 1)
                def _():
                    step(i + 1, s0, m0, kb0, kr0, i, s1, m1, nn, kb1, kr1)
                return carry
            lax.fori_loop(0, H - 1, body, 0)
            sl, ml = (s0, m0) if (H - 1) % 2 == 0 else (s1, m1)
            step(None, None, None, None, None, H - 1, sl, ml, None, None, None)

        def post_tiles(r0s):
            x1s = []
            for r0 in r0s:
                rows = pl.ds(r0, TS)
                attn = lax.dot_general(ot[:, rows], wo[...], (((0,), (0,)), ((), ())),
                                       preferred_element_type=F32)
                x1s.append(x[rows, :] + attn)
            x2s = []
            for x1 in x1s:
                xn = _layernorm(x1).astype(BF16)
                hid = jnp.dot(xn, w1[...], preferred_element_type=F32) + b1[...].astype(F32)
                hid = _gelu_tanh(hid).astype(BF16)
                y = jnp.dot(hid, w2[...], preferred_element_type=F32) + b2[...].astype(F32)
                x2s.append(x1 + y)
            return x2s

        layer = pl.program_id(0)

        @pl.when(layer == 0)
        def _():
            wqkv_copy.start()
            x_copy(0).start()
            wqkv_copy.wait()
            for t in range(1, nt):
                x_copy(t).start()
            wqvt[0:D, :] = wqkv[:, 0:D].astype(F32).T.astype(BF16)
            wqvt[D:2 * D, :] = wqkv[:, 2 * D:3 * D].astype(F32).T.astype(BF16)

            def body(t, carry):
                x_copy(t).wait()
                for r0 in subrows(t):
                    xt = x_in[pl.ds(r0, TS), :].astype(F32)
                    x[pl.ds(r0, TS), :] = xt
                    qkv_mm(r0, _layernorm(xt).astype(BF16))
                return carry
            lax.fori_loop(0, nt, body, 0)
            for c in late_copies:
                c.start()

        attention()

        @pl.when(layer == 0)
        def _():
            for c in late_copies:
                c.wait()

            def body(t, carry):
                rl = subrows(t)
                for r0, x2 in zip(rl, post_tiles(rl)):
                    x[pl.ds(r0, TS), :] = x2
                    qkv_mm(r0, _layernorm(x2).astype(BF16))
                return carry
            lax.fori_loop(0, nt, body, 0)

        @pl.when(layer == 1)
        def _():
            def body(t, carry):
                rl = subrows(t)
                for r0, x2 in zip(rl, post_tiles(rl)):
                    out[pl.ds(r0, TS), :] = x2.astype(out.dtype)
                out_copy(t).start()
                return carry
            lax.fori_loop(0, nt, body, 0)
            for t in range(nt):
                out_copy(t).wait()

    scratch = [
        pltpu.VMEM((S, D), BF16),
        pltpu.VMEM((D, 3 * D), BF16),
        pltpu.VMEM((D, D), BF16),
        pltpu.VMEM((D, F), BF16),
        pltpu.VMEM((F, D), BF16),
        pltpu.VMEM((S, D), BF16),
        pltpu.VMEM((S, D), F32),
        pltpu.VMEM((2 * D, D), BF16),
        pltpu.VMEM((D // 2, S), U32),
        pltpu.VMEM((S // 2, D), U32),
        pltpu.VMEM((D // 2, S), U32),
        pltpu.VMEM((D, S), BF16),
        pltpu.VMEM((nq, S, TQ), F32),
        pltpu.VMEM((nq, S, TQ), F32),
        pltpu.VMEM((nq, 8, TQ), F32),
        pltpu.VMEM((nq, 8, TQ), F32),
        pltpu.VMEM((DH, S), F32),
        pltpu.VMEM((DH, ngrp * 128, 128), F32),
        pltpu.VMEM((DH, ngrp * 128, 128), F32),
        pltpu.VMEM((S // 2, 128), U32),
        pltpu.VMEM((S // 2, 128), U32),
        pltpu.VMEM((ngrp, H, DH, 128), F32),
        pltpu.SemaphoreType.DMA((nt,)),
        pltpu.SemaphoreType.DMA((4,)),
        pltpu.SemaphoreType.DMA((nt,)),
    ]
    return kernel, scratch


@jax.jit
def pallas_interleave_layers__mha_block__dense_activation_gelu__prompt_kernel(
    A_x: jax.Array,
    A_wqkv: jax.Array,
    A_wo: jax.Array,
    B_x: jax.Array,
    B_w1: jax.Array,
    B_b1: jax.Array,
    B_w2: jax.Array,
    B_b2: jax.Array,
):
    B, S, D = A_x.shape
    F = B_w1.shape[1]
    assert B == 1
    x2d = A_x.reshape(S, D)

    def full(shape):
        return pl.BlockSpec(shape, lambda i: (0,) * len(shape))

    hbm = pl.BlockSpec(memory_space=pl.ANY)
    kernel, scratch = _make_kernel(S, D, F)

    out = pl.pallas_call(
        kernel,
        grid=(2,),
        in_specs=[hbm, hbm, hbm, hbm, full((F,)), hbm, full((D,))],
        out_specs=hbm,
        out_shape=jax.ShapeDtypeStruct((S, D), A_x.dtype),
        scratch_shapes=scratch,
        compiler_params=pltpu.CompilerParams(
            dimension_semantics=("arbitrary",),
            vmem_limit_bytes=100 * 1024 * 1024,
        ),
    )(x2d, A_wqkv, A_wo, B_w1, B_b1, B_w2, B_b2)
    return out.reshape(B, S, D)
```

```python
import math

import jax
import jax.numpy as jnp
from jax import lax
import jax.experimental.pallas as pl
import jax.experimental.pallas.tpu as pltpu

F32 = jnp.float32
BF16 = jnp.bfloat16
U32 = jnp.uint32

N_HEADS = 32
LN_EPS = 1e-5
TQ = 512
CK = 128
TS = 128
TM = 256
TM_LAST = 512
TE = 128
GV = 21
GV0 = 19
L_LO = 2.0 ** -60
L_HI = 2.0 ** 57
V_HI = 2.0 ** 60


def _layernorm(x):
    m = jnp.mean(x, axis=-1, keepdims=True)
    xc = x - m
    v = jnp.mean(xc * xc, axis=-1, keepdims=True)
    return xc * lax.rsqrt(v + LN_EPS)


def _gelu_tanh(x):
    c = math.sqrt(2.0 / math.pi)
    return 0.5 * x * (1.0 + jnp.tanh(c * (x + 0.044715 * (x * x * x))))


def _dot(a, b, dims=(((1,), (0,)), ((), ()))):
    return lax.dot_general(a, b, dims, precision=lax.Precision.DEFAULT,
                           preferred_element_type=F32)


def _make_kernel(S, D, F):
    H = N_HEADS
    DH = D // H
    HPG = 128 // DH
    nslab = D // 128
    nq = S // TQ
    nck = S // CK
    nt = S // TM
    ntl = TQ // 128
    nsteps = nq * nck
    qscale = (DH ** -0.5) * math.log2(math.e)
    ngrp = (GV * 16 + 127) // 128
    ngrp0 = (GV0 * 16 + 127) // 128
    assert nt == 2 * nslab and ngrp * 128 <= nslab * TM and DH % nslab == 0

    def plan(g):
        nm = S // 16 - g
        segs = [(nm * (c + 1)) // nck - (nm * c) // nck for c in range(nck)]
        pieces = sorted([(i, t) for i in range(g) for t in range(ntl)],
                        key=lambda p: ((p[0] + 5 * p[1]) % g, p[1]))
        pos = {}
        for n, p in enumerate(pieces):
            pos.setdefault(int((n + 0.5) * 2 * nm / len(pieces)), []).append(p)
        return segs, pos

    tr_pos = {}
    for n in range(DH * ngrp):
        tr_pos.setdefault(n * nsteps // (DH * ngrp), []).append(n)

    def kernel(x_hbm, wqkv_hbm, wo_hbm, w1_hbm, b1_hbm, w2_hbm, b2_hbm, out_hbm,
               x_in, wqkv, wo, w1, w2, out,
               x, qt, qf, k, vt, ot, on, ls, p0, p1, kb0, kb1, kr0, kr1, qs0, qs1,
               kto, kbz, kt0, rng, b1, b2, xsem, wsem, osem):
        layer = pl.program_id(0)

        def x_copy(t):
            return pltpu.make_async_copy(x_hbm.at[pl.ds(t * TM, TM), :],
                                         x_in.at[pl.ds(t * TM, TM), :], xsem.at[t])

        def out_copy(t):
            return pltpu.make_async_copy(out.at[pl.ds(t * TS, TS), :],
                                         out_hbm.at[pl.ds(t * TS, TS), :], osem.at[0])

        wqkv_copy = pltpu.make_async_copy(wqkv_hbm, wqkv, wsem.at[0])
        late_copies = [pltpu.make_async_copy(src, dst, wsem.at[1])
                       for src, dst in ((wo_hbm, wo), (w1_hbm, w1), (w2_hbm, w2),
                                        (b1_hbm, b1), (b2_hbm, b2))]

        def rng_reset():
            rng[0] = jnp.full((8, 128), L_HI, F32)
            rng[1] = jnp.full((8, 128), L_LO, F32)
            rng[2] = jnp.zeros((8, 128), F32)

        def qkv_mm(r0, xn):
            rows = pl.ds(r0, TS)
            tt_dims = (((0,), (1,)), ((), ()))
            kk = pltpu.bitcast(_dot(xn, wqkv[:, D:2 * D]).astype(BF16), U32)
            for g in range(nslab):
                k[g, pl.ds(pl.multiple_of(r0 // 2, TS // 2), TS // 2), :] = (
                    kk[:, g * 128:(g + 1) * 128])
            q = _dot(wqkv[:, 0:D], xn, tt_dims) * qscale
            qt[:, :, rows] = pltpu.bitcast(q.astype(BF16), U32).reshape(H, DH // 2, TS)
            qf[:, :, rows] = q.reshape(H, DH, TS)
            v = _dot(wqkv[:, 2 * D:3 * D], xn, tt_dims)
            vt[:, :, rows] = v.reshape(H, DH, TS)
            rng[2] = jnp.maximum(rng[2], jnp.max(jnp.abs(v).reshape(D // 8, 8, TS), axis=0))

        def subrows(t, tm):
            return [pl.multiple_of(t * tm + i * TS, TS) for i in range(tm // TS)]

        def k_rot(h, r0, nr):
            kc = k[h // HPG, pl.ds(r0, nr), :]
            return pltpu.roll(kc, (128 - (h % HPG) * DH) % 128, 1)

        def prep(h, n, kb, kr, qs, hist, lag, off):
            nr = (S // 2) // nsteps
            if (n + 1) * nr * 2 > 16 * GV:
                kr[pl.ds(n * nr, nr), :] = k_rot(h, n * nr, nr)
            if n % 4 == 1:
                cols = pl.ds((n // 4) * 128, 128)
                qs[:, cols] = qf[h, :, cols]
            for idx in tr_pos.get(n, []):
                gi, d = idx // DH, idx % DH
                nk = min(128, GV * 16 - gi * 128)
                row = jnp.broadcast_to(kto[h, gi, d:d + 1, :], (8, 128))
                if len(hist) >= lag:
                    never = lax.broadcasted_iota(jnp.int32, (8, 128), 1) < -1 - layer
                    row = jnp.where(never, hist[-lag], row)
                v = jnp.concatenate([row] * 16, axis=0).T
                kb[d, gi * 128:gi * 128 + nk, :] = v[:nk]
                hist.append(v[off:off + 8])

        def prep_tables(t):
            nd = DH // nslab
            sl = t % nslab
            for gi in range(ngrp0):
                kt = pltpu.bitcast(k[0, gi * 64:(gi + 1) * 64, :], BF16).astype(F32).T
                kt0[gi] = kt[0:DH]
            for gi in range(ngrp):
                kt = pltpu.bitcast(k[sl, gi * 64:(gi + 1) * 64, :], BF16).astype(F32).T
                kto[pl.ds(sl * HPG, HPG), gi] = kt.reshape(HPG, DH, 128)
            for gi in range(ngrp0):
                nk = min(128, GV0 * 16 - gi * 128)
                for e in range(nd):
                    d = sl * nd + e
                    row = kt0[gi, pl.ds(d, 1), :]
                    kbz[d, gi * 128:gi * 128 + nk, :] = (
                        jnp.broadcast_to(row, (128, 128)).T[:nk])

        def piece(p, kba, qs, pbuf, j, l):
            i, t = p
            c0 = j * TQ + t * 128
            accs = {}
            for d in range(DH):
                qb = jnp.broadcast_to(qs[d:d + 1, c0:c0 + 128], (8, 128))
                for r in range(2):
                    o = 16 * i + r * 8
                    pr = kba[d, o:o + 8, :] * qb
                    key = (r, d % 2)
                    accs[key] = accs[key] + pr if key in accs else pr
            for r in range(2):
                e = jnp.exp2(accs[r, 0] + accs[r, 1])
                l[t] = l[t] + e
                pbuf[j, pl.ds(16 * i + r * 8, 8), t * 128:(t + 1) * 128] = e

        def normalize(h, cols, o):
            lsum = jnp.sum(ls[h, :, cols], axis=0, keepdims=True)
            r0 = pl.reciprocal(lsum, approx=True)
            rinv = r0 * (2.0 - lsum * r0)
            on[h * DH:(h + 1) * DH, cols] = (o * rinv).astype(BF16)

        def step(ha, pa, kba, kra, qsa, hb, pb, hn, kbn, krn, qsn):
            gv = GV0 if hb is None else GV
            segs, pos = plan(gv)
            hist = []
            for j in range(nq):
                if ha is not None:
                    w = pltpu.bitcast(qt[ha, :, pl.ds(j * TQ, TQ)], BF16)
                acc = None
                l = [None] * ntl
                g0 = gv
                for c in range(nck):
                    if ha is not None:
                        nm = segs[c] * 16
                        kc = pltpu.bitcast(kra[pl.ds(g0 * 8, nm // 2), :], BF16)
                        p = jnp.exp2(_dot(kc[:, 0:DH], w))
                        pa[j, pl.ds(g0 * 16, nm), :] = p
                        for r in range(nm // 8):
                            for t in range(ntl):
                                pr = p[r * 8:(r + 1) * 8, t * 128:(t + 1) * 128]
                                l[t] = pr if l[t] is None else l[t] + pr
                            for pc in pos.get((g0 - gv) * 2 + r, []):
                                piece(pc, kba, qsa, pa, j, l)
                        g0 += segs[c]
                    if hb is not None:
                        o = _dot(vt[hb, :, pl.ds(c * CK, CK)], pb[j, pl.ds(c * CK, CK), :])
                        acc = o if acc is None else o + acc
                    if hn is not None:
                        prep(hn, j * nck + c, kbn, krn, qsn, hist,
                             *((2, 64) if hb is None else (1, 0)))
                    if ha is None:
                        n = j * nck + c
                        hd, part = n * H // nsteps, n % (nsteps // H)
                        cw = S * H // nsteps
                        if hd != hb:
                            cols = pl.ds(part * cw, cw)
                            normalize(hd, cols, ot[hd, :, cols])
                if ha is None:
                    normalize(hb, pl.ds(j * TQ, TQ), acc)
                elif hb is not None:
                    ot[hb, :, pl.ds(j * TQ, TQ)] = acc
                if ha is not None:
                    ls[ha, :, pl.ds(j * TQ, TQ)] = jnp.concatenate(l, axis=1)
                    rng[0] = jnp.minimum(rng[0], jnp.minimum(jnp.minimum(l[0], l[1]),
                                                             jnp.minimum(l[2], l[3])))
                    rng[1] = jnp.maximum(rng[1], jnp.maximum(jnp.maximum(l[0], l[1]),
                                                             jnp.maximum(l[2], l[3])))

        def exact_attention():
            ne = S // TE

            def body(u, carry):
                h = u // ne
                cols = pl.ds(pl.multiple_of((u % ne) * TE, TE), TE)
                w = pltpu.bitcast(qt[h, :, cols], BF16)
                kc = pltpu.bitcast(k_rot(h, 0, S // 2), BF16)
                s = _dot(kc[:, 0:DH], w)
                p = jnp.exp2(s - jnp.max(s, axis=0, keepdims=True))
                o = _dot(vt[h], p) / jnp.sum(p, axis=0, keepdims=True)
                on[pl.ds(pl.multiple_of(h * DH, DH), DH), cols] = o.astype(BF16)
                return carry
            lax.fori_loop(0, H * ne, body, 0)

        def attention():
            step(0, p0, kbz, k.at[0], qf.at[0], None, None, 1, kb1, kr1, qs1)

            def body(i, carry):
                h = 2 * i
                step(h + 1, p1, kb1, kr1, qs1, h, p0,
                     jnp.minimum(h + 2, H - 1), kb0, kr0, qs0)

                @pl.when(h + 2 < H)
                def _():
                    step(h + 2, p0, kb0, kr0, qs0, h + 1, p1, h + 3, kb1, kr1, qs1)
                return carry
            lax.fori_loop(0, H // 2, body, 0)
            ok = (rng[0] >= L_LO) & (rng[1] <= L_HI) & (rng[2] <= V_HI)
            nbad = jnp.max(jnp.where(ok, 0.0, 1.0))
            rng_reset()
            step(None, None, None, None, None, H - 1, p1, None, None, None, None)

            @pl.when(nbad > 0.0)
            def _():
                exact_attention()

        def o_first(t, tm):
            r0 = pl.multiple_of(jnp.minimum(t, S // tm - 1) * tm, tm)
            return on[:, pl.ds(r0, TS)].T

        def post_tiles(r0s, o0):
            x1s = []
            for n, r0 in enumerate(r0s):
                if n == 0:
                    attn = _dot(o0, wo[...])
                else:
                    attn = _dot(on[:, pl.ds(r0, TS)], wo[...], (((0,), (0,)), ((), ())))
                x1s.append(x[pl.ds(r0, TS), :] + attn)
            x2s = []
            for x1 in x1s:
                xn = _layernorm(x1).astype(BF16)
                hid = _dot(xn, w1[...]) + b1[...].astype(F32)
                hid = _gelu_tanh(hid).astype(BF16)
                y = _dot(hid, w2[...]) + b2[...].astype(F32)
                x2s.append(x1 + y)
            return x2s

        @pl.when(layer == 0)
        def _():
            x_copy(0).start()
            wqkv_copy.start()
            x_copy(1).start()
            rng_reset()
            k[:, 0:ngrp * 64, :] = jnp.zeros((nslab, ngrp * 64, 128), U32)

            def ln_first(t):
                r0 = pl.multiple_of(jnp.minimum(t, nt - 1) * TM, TM)
                return _layernorm(x_in[pl.ds(r0, TS), :].astype(F32)).astype(BF16)

            x_copy(0).wait()
            xn0 = ln_first(0)
            wqkv_copy.wait()
            for t in range(2, nt):
                x_copy(t).start()

            def body(t, xn0):
                @pl.when(t + 1 < nt)
                def _():
                    x_copy(t + 1).wait()

                prep_tables(t)
                for n, r0 in enumerate(subrows(t, TM)):
                    xt = x_in[pl.ds(r0, TS), :].astype(F32)
                    x[pl.ds(r0, TS), :] = xt
                    qkv_mm(r0, xn0 if n == 0 else _layernorm(xt).astype(BF16))
                return ln_first(t + 1)
            lax.fori_loop(0, nt, body, xn0)
            for c in late_copies:
                c.start()

        attention()

        @pl.when(layer == 0)
        def _():
            for c in late_copies:
                c.wait()

            def body(t, o0):
                rl = subrows(t, TM)
                prep_tables(t)
                for r0, x2 in zip(rl, post_tiles(rl, o0)):
                    x[pl.ds(r0, TS), :] = x2
                    qkv_mm(r0, _layernorm(x2).astype(BF16))
                return o_first(t + 1, TM)
            lax.fori_loop(0, nt, body, o_first(0, TM))

        @pl.when(layer == 1)
        def _():
            def body(t, o0):
                rl = subrows(t, TM_LAST)
                for n, (r0, x2) in enumerate(zip(rl, post_tiles(rl, o0))):
                    out[pl.ds(r0, TS), :] = x2.astype(out.dtype)
                    out_copy(t * (TM_LAST // TS) + n).start()
                return o_first(t + 1, TM_LAST)
            lax.fori_loop(0, S // TM_LAST, body, o_first(0, TM_LAST))
            for t in range(S // TS):
                out_copy(t).wait()

    scratch = [
        pltpu.VMEM((S, D), BF16),
        pltpu.VMEM((D, 3 * D), BF16),
        pltpu.VMEM((D, D), BF16),
        pltpu.VMEM((D, F), BF16),
        pltpu.VMEM((F, D), BF16),
        pltpu.VMEM((S, D), BF16),
        pltpu.VMEM((S, D), F32),
        pltpu.VMEM((H, DH // 2, S), U32),
        pltpu.VMEM((H, DH, S), F32),
        pltpu.VMEM((nslab, S // 2, 128), U32),
        pltpu.VMEM((H, DH, S), F32),
        pltpu.VMEM((H, DH, S), F32),
        pltpu.VMEM((D, S), BF16),
        pltpu.VMEM((H, 8, S), F32),
        pltpu.VMEM((nq, S, TQ), F32),
        pltpu.VMEM((nq, S, TQ), F32),
        pltpu.VMEM((DH, ngrp * 128, 128), F32),
        pltpu.VMEM((DH, ngrp * 128, 128), F32),
        pltpu.VMEM((S // 2, 128), U32),
        pltpu.VMEM((S // 2, 128), U32),
        pltpu.VMEM((DH, S), F32),
        pltpu.VMEM((DH, S), F32),
        pltpu.VMEM((H, 4, DH, 128), F32),
        pltpu.VMEM((DH, ngrp0 * 128 + 8, 128), F32),
        pltpu.VMEM((4, DH, 128), F32),
        pltpu.VMEM((4, 8, 128), F32),
        pltpu.VMEM((F,), BF16),
        pltpu.VMEM((D,), BF16),
        pltpu.SemaphoreType.DMA((nt,)),
        pltpu.SemaphoreType.DMA((2,)),
        pltpu.SemaphoreType.DMA((1,)),
    ]
    return kernel, scratch


@jax.jit
def pallas_interleave_layers__mha_block__dense_activation_gelu__prompt_kernel(
    A_x: jax.Array,
    A_wqkv: jax.Array,
    A_wo: jax.Array,
    B_x: jax.Array,
    B_w1: jax.Array,
    B_b1: jax.Array,
    B_w2: jax.Array,
    B_b2: jax.Array,
):
    B, S, D = A_x.shape
    F = B_w1.shape[1]
    assert B == 1
    x2d = A_x.reshape(S, D)

    hbm = pl.BlockSpec(memory_space=pl.ANY)
    kernel, scratch = _make_kernel(S, D, F)

    out = pl.pallas_call(
        kernel,
        grid=(2,),
        in_specs=[hbm] * 7,
        out_specs=hbm,
        out_shape=jax.ShapeDtypeStruct((S, D), A_x.dtype),
        scratch_shapes=scratch,
        compiler_params=pltpu.CompilerParams(
            dimension_semantics=("arbitrary",),
            vmem_limit_bytes=100 * 1024 * 1024,
        ),
    )(x2d, A_wqkv, A_wo, B_w1, B_b1, B_w2, B_b2)
    return out.reshape(B, S, D)
```

```python
import math

import jax
import jax.numpy as jnp
from jax import lax
import jax.experimental.pallas as pl
import jax.experimental.pallas.tpu as pltpu

F32 = jnp.float32
BF16 = jnp.bfloat16
U32 = jnp.uint32

N_HEADS = 32
LN_EPS = 1e-5
TQ = 512
CK = 128
TS = 128
TM = 256
TM_LAST = 256
TE = 128
GV = 21
GV0 = 19
L_LO = 2.0 ** -60
L_HI = 2.0 ** 57
V_HI = 2.0 ** 60


def _layernorm(x):
    m = jnp.mean(x, axis=-1, keepdims=True)
    xc = x - m
    v = jnp.mean(xc * xc, axis=-1, keepdims=True)
    return xc * lax.rsqrt(v + LN_EPS)


def _gelu_tanh(x):
    c = math.sqrt(2.0 / math.pi)
    return 0.5 * x * (1.0 + jnp.tanh(c * (x + 0.044715 * (x * x * x))))


def _dot(a, b, dims=(((1,), (0,)), ((), ()))):
    return lax.dot_general(a, b, dims, precision=lax.Precision.DEFAULT,
                           preferred_element_type=F32)


def _make_kernel(S, D, F):
    H = N_HEADS
    DH = D // H
    HPG = 128 // DH
    nslab = D // 128
    nq = S // TQ
    nck = S // CK
    nt = S // TM
    ntl = TQ // 128
    nsteps = nq * nck
    qscale = (DH ** -0.5) * math.log2(math.e)
    ngrp = (GV * 16 + 127) // 128
    ngrp0 = (GV0 * 16 + 127) // 128
    assert nt == 2 * nslab and ngrp * 128 <= nslab * TM and DH % nslab == 0

    def plan(g):
        nm = S // 16 - g
        segs = [(nm * (c + 1)) // nck - (nm * c) // nck for c in range(nck)]
        pieces = sorted([(i, t) for i in range(g) for t in range(ntl)],
                        key=lambda p: ((p[0] + 5 * p[1]) % g, p[1]))
        pos = {}
        for n, p in enumerate(pieces):
            pos.setdefault(int((n + 0.5) * 2 * nm / len(pieces)), []).append(p)
        return segs, pos

    tr_pos = {}
    for n in range(DH * ngrp):
        tr_pos.setdefault(n * nsteps // (DH * ngrp), []).append(n)

    def kernel(x_hbm, wqkv_hbm, wo_hbm, w1_hbm, b1_hbm, w2_hbm, b2_hbm, out_hbm,
               x_in, wqkv, wo, w1, w2, out,
               x, qt, qf, k, vt, ot, on, ls, p0, p1, kb0, kb1, kr0, kr1, qs0, qs1,
               kto, kbz, kt0, o0buf, w1s, w2s, rng, b1, b2, xsem, wsem, osem):
        layer = pl.program_id(0)

        def x_copy(t):
            return pltpu.make_async_copy(x_hbm.at[pl.ds(t * TM, TM), :],
                                         x_in.at[pl.ds(t * TM, TM), :], xsem.at[t])

        def out_copy(t):
            return pltpu.make_async_copy(out.at[pl.ds(t * TS, TS), :],
                                         out_hbm.at[pl.ds(t * TS, TS), :], osem.at[0])

        wqkv_copies = [pltpu.make_async_copy(wqkv_hbm.at[:, pl.ds(c * D, D)],
                                             wqkv.at[:, pl.ds(c * D, D)], wsem.at[1 + c])
                       for c in (1, 0, 2)]
        ffn_copies = [pltpu.make_async_copy(src, dst, wsem.at[0])
                      for src, dst in ((w1_hbm, w1), (w2_hbm, w2))]
        late_copies = [pltpu.make_async_copy(src, dst, wsem.at[0])
                       for src, dst in ((wo_hbm, wo), (b1_hbm, b1), (b2_hbm, b2))]

        def rng_reset():
            rng[0] = jnp.full((8, 128), L_HI, F32)
            rng[1] = jnp.full((8, 128), L_LO, F32)
            rng[2] = jnp.zeros((8, 128), F32)

        tt_dims = (((0,), (1,)), ((), ()))

        def k_mm(r0, xn):
            kf = _dot(xn, wqkv[:, D:2 * D])
            kk = pltpu.bitcast(kf.astype(BF16), U32)
            for g in range(nslab):
                k[g, pl.ds(pl.multiple_of(r0 // 2, TS // 2), TS // 2), :] = (
                    kk[:, g * 128:(g + 1) * 128])
            return [kf[r:r + 8, c:c + 128] for c in range(0, D, 128) for r in range(0, TS, 8)]

        def q_mm(r0, xn):
            rows = pl.ds(r0, TS)
            q = _dot(wqkv[:, 0:D], xn, tt_dims) * qscale
            qt[:, :, rows] = pltpu.bitcast(q.astype(BF16), U32).reshape(H, DH // 2, TS)
            qf[:, :, rows] = q.reshape(H, DH, TS)
            return [q[r:r + 8] for r in range(0, D, 8)]

        def v_mm(r0, xn):
            v = _dot(wqkv[:, 2 * D:3 * D], xn, tt_dims)
            vt[:, :, pl.ds(r0, TS)] = v.reshape(H, DH, TS)
            rng[2] = jnp.maximum(rng[2], jnp.max(jnp.abs(v).reshape(D // 8, 8, TS), axis=0))
            return [v[r:r + 8] for r in range(0, D, 8)]

        def qkv_mm(r0, xn):
            return k_mm(r0, xn) + q_mm(r0, xn) + v_mm(r0, xn)

        def subrows(t, tm):
            return [pl.multiple_of(t * tm + i * TS, TS) for i in range(tm // TS)]

        def k_rot(h, r0, nr):
            kc = k[h // HPG, pl.ds(r0, nr), :]
            return pltpu.roll(kc, (128 - (h % HPG) * DH) % 128, 1)

        def prep(h, n, kb, kr, qs, hist, lag, off):
            nr = (S // 2) // nsteps
            if (n + 1) * nr * 2 > 16 * GV:
                kr[pl.ds(n * nr, nr), :] = k_rot(h, n * nr, nr)
            if n % 4 == 1:
                cols = pl.ds((n // 4) * 128, 128)
                qs[:, cols] = qf[h, :, cols]
            for idx in tr_pos.get(n, []):
                gi, d = idx // DH, idx % DH
                nk = min(128, GV * 16 - gi * 128)
                row = jnp.broadcast_to(kto[h, gi, d:d + 1, :], (8, 128))
                if len(hist) >= lag:
                    never = lax.broadcasted_iota(jnp.int32, (8, 128), 1) < -1 - layer
                    row = jnp.where(never, hist[-lag], row)
                v = jnp.concatenate([row] * 16, axis=0).T
                kb[d, gi * 128:gi * 128 + nk, :] = v[:nk]
                hist.append(v[off:off + 8])

        def prep_tables(t):
            nd = DH // nslab
            sl = t % nslab
            for gi in range(ngrp0):
                kt = pltpu.bitcast(k[0, gi * 64:(gi + 1) * 64, :], BF16).astype(F32).T
                kt0[gi] = kt[0:DH]
            for gi in range(ngrp):
                kt = pltpu.bitcast(k[sl, gi * 64:(gi + 1) * 64, :], BF16).astype(F32).T
                kto[pl.ds(sl * HPG, HPG), gi] = kt.reshape(HPG, DH, 128)
            for gi in range(ngrp0):
                nk = min(128, GV0 * 16 - gi * 128)
                for e in range(nd):
                    d = sl * nd + e
                    row = kt0[gi, pl.ds(d, 1), :]
                    kbz[d, gi * 128:gi * 128 + nk, :] = (
                        jnp.broadcast_to(row, (128, 128)).T[:nk])

        def piece(p, kba, qs, pbuf, j, l):
            i, t = p
            c0 = j * TQ + t * 128
            accs = {}
            for d in range(DH):
                qb = jnp.broadcast_to(qs[d:d + 1, c0:c0 + 128], (8, 128))
                for r in range(2):
                    o = 16 * i + r * 8
                    pr = kba[d, o:o + 8, :] * qb
                    key = (r, d % 2)
                    accs[key] = accs[key] + pr if key in accs else pr
            for r in range(2):
                e = jnp.exp2(accs[r, 0] + accs[r, 1])
                l[t] = l[t] + e
                pbuf[j, pl.ds(16 * i + r * 8, 8), t * 128:(t + 1) * 128] = e

        def normalize(h, cols, o):
            lsum = jnp.sum(ls[h, :, cols], axis=0, keepdims=True)
            r0 = pl.reciprocal(lsum, approx=True)
            rinv = r0 * (2.0 - lsum * r0)
            on[h * DH:(h + 1) * DH, cols] = (o * rinv).astype(BF16)

        def step(ha, pa, kba, kra, qsa, hb, pb, hn, kbn, krn, qsn):
            gv = GV0 if hb is None else GV
            segs, pos = plan(gv)
            hist = []
            for j in range(nq):
                if ha is not None:
                    w = pltpu.bitcast(qt[ha, :, pl.ds(j * TQ, TQ)], BF16)
                acc = None
                l = [None] * ntl
                g0 = gv
                for c in range(nck):
                    if ha is not None:
                        nm = segs[c] * 16
                        kc = pltpu.bitcast(kra[pl.ds(g0 * 8, nm // 2), :], BF16)
                        p = jnp.exp2(_dot(kc[:, 0:DH], w))
                        pa[j, pl.ds(g0 * 16, nm), :] = p
                        for r in range(nm // 8):
                            for t in range(ntl):
                                pr = p[r * 8:(r + 1) * 8, t * 128:(t + 1) * 128]
                                l[t] = pr if l[t] is None else l[t] + pr
                            for pc in pos.get((g0 - gv) * 2 + r, []):
                                piece(pc, kba, qsa, pa, j, l)
                        g0 += segs[c]
                    if hb is not None:
                        o = _dot(vt[hb, :, pl.ds(c * CK, CK)], pb[j, pl.ds(c * CK, CK), :])
                        acc = o if acc is None else o + acc
                    if hn is not None:
                        prep(hn, j * nck + c, kbn, krn, qsn, hist,
                             *((2, 64) if hb is None else (1, 0)))
                    if ha is None:
                        n = j * nck + c
                        hd, part = n % H, n // H
                        cw = S * H // nsteps
                        if hd != hb:
                            cols = pl.ds(part * cw, cw)
                            normalize(hd, cols, ot[hd, :, cols])
                        if n == H + 8:
                            o0buf[...] = pltpu.bitcast(on[:, 0:TS].T, U32)
                if ha is None:
                    normalize(hb, pl.ds(j * TQ, TQ), acc)
                elif hb is not None:
                    ot[hb, :, pl.ds(j * TQ, TQ)] = acc
                if ha is not None:
                    ls[ha, :, pl.ds(j * TQ, TQ)] = jnp.concatenate(l, axis=1)
                    rng[0] = jnp.minimum(rng[0], jnp.minimum(jnp.minimum(l[0], l[1]),
                                                             jnp.minimum(l[2], l[3])))
                    rng[1] = jnp.maximum(rng[1], jnp.maximum(jnp.maximum(l[0], l[1]),
                                                             jnp.maximum(l[2], l[3])))

        def exact_attention():
            ne = S // TE

            def body(u, carry):
                h = u // ne
                cols = pl.ds(pl.multiple_of((u % ne) * TE, TE), TE)
                w = pltpu.bitcast(qt[h, :, cols], BF16)
                kc = pltpu.bitcast(k_rot(h, 0, S // 2), BF16)
                s = _dot(kc[:, 0:DH], w)
                p = jnp.exp2(s - jnp.max(s, axis=0, keepdims=True))
                o = _dot(vt[h], p) / jnp.sum(p, axis=0, keepdims=True)
                on[pl.ds(pl.multiple_of(h * DH, DH), DH), cols] = o.astype(BF16)
                return carry
            lax.fori_loop(0, H * ne, body, 0)
            o0buf[...] = pltpu.bitcast(on[:, 0:TS].T, U32)

        def attention():
            step(0, p0, kbz, k.at[0], qf.at[0], None, None, 1, kb1, kr1, qs1)

            def body(i, carry):
                h = 2 * i
                step(h + 1, p1, kb1, kr1, qs1, h, p0,
                     jnp.minimum(h + 2, H - 1), kb0, kr0, qs0)

                @pl.when(h + 2 < H)
                def _():
                    step(h + 2, p0, kb0, kr0, qs0, h + 1, p1, h + 3, kb1, kr1, qs1)
                return carry
            lax.fori_loop(0, H // 2, body, 0)
            ok = (rng[0] >= L_LO) & (rng[1] <= L_HI) & (rng[2] <= V_HI)
            nbad = jnp.max(jnp.where(ok, 0.0, 1.0))
            rng_reset()
            step(None, None, None, None, None, H - 1, p1, None, None, None, None)

            @pl.when(nbad > 0.0)
            def _():
                exact_attention()

        def strassen(a11, a12, a21, a22, ws, order):
            lhs = {1: lambda: a11 + a22, 2: lambda: a21 + a22, 3: lambda: a11, 4: lambda: a22,
                   5: lambda: a11 + a12, 6: lambda: a21 - a11, 7: lambda: a12 - a22}
            m = {i: _dot(lhs[i]().astype(BF16), pltpu.bitcast(ws[i - 1], BF16)) for i in order}
            terms = (((1, 1), (4, 1), (5, -1), (7, 1)), ((3, 1), (5, 1)),
                     ((2, 1), (4, 1)), ((1, 1), (2, -1), (3, 1), (6, 1)))
            outs = []
            for ts in terms:
                ts = sorted(ts, key=lambda t: order.index(t[0]))
                if ts[0][1] < 0:
                    ts[0], ts[1] = ts[1], ts[0]
                acc = m[ts[0][0]]
                for i, sg in ts[1:]:
                    acc = acc + m[i] if sg > 0 else acc - m[i]
                outs.append(acc)
            return outs

        def strassen_weights(w, ws, swap, r0, c0, tie):
            kh, nh = w.shape[0] // 2, w.shape[1] // 2
            never = lax.broadcasted_iota(jnp.int32, (8, 128), 1) < -1 - layer
            tie = pltpu.bitcast(tie, U32)

            def blk(r, c):
                v = pltpu.bitcast(w[pl.ds(r + r0, 16), c + c0:c + c0 + 128], U32)
                return pltpu.bitcast(jnp.where(never, tie, v), BF16)
            b11, b12, b21, b22 = blk(0, 0), blk(0, nh), blk(kh, 0), blk(kh, nh)
            if swap:
                b11, b12, b21, b22 = b21, b22, b11, b12
            f11, f12, f21, f22 = [b.astype(F32) for b in (b11, b12, b21, b22)]
            rows = pl.ds(pl.multiple_of(r0 // 2, 8), 8)
            for n, v in enumerate((f11 + f22, b11, f12 - f22, f21 - f11, b22,
                                   f11 + f12, f21 + f22)):
                ws[n, rows, c0:c0 + 128] = pltpu.bitcast(v.astype(BF16), U32)

        def o_first(t, tm):
            r0 = pl.multiple_of(jnp.minimum(t, S // tm - 1) * tm, tm)
            return on[:, pl.ds(r0, TS)].T

        def post_tiles(r0s, o0):
            x1s = []
            for n, r0 in enumerate(r0s):
                if n == 0:
                    attn = _dot(o0, wo[...])
                else:
                    attn = _dot(on[:, pl.ds(r0, TS)], wo[...], (((0,), (0,)), ((), ())))
                x1s.append(x[pl.ds(r0, TS), :] + attn)
            top, bot = [_layernorm(x1) for x1 in x1s]
            b1f = b1[...].astype(F32)
            b2f = b2[...].astype(F32)
            c = strassen(top[:, :D // 2], top[:, D // 2:], bot[:, :D // 2], bot[:, D // 2:],
                         w1s, (3, 5, 2, 4, 1, 7, 6))
            h11, h12, h21, h22 = [_gelu_tanh(ci + bi) for ci, bi in zip(
                c, (b1f[:F // 2], b1f[F // 2:]) * 2)]
            c = strassen(h12, h11, h22, h21, w2s, (3, 4, 1, 5, 7, 2, 6))
            return [x1s[0] + (jnp.concatenate(c[0:2], axis=1) + b2f),
                    x1s[1] + (jnp.concatenate(c[2:4], axis=1) + b2f)]

        @pl.when(layer < 1)
        def _():
            x_copy(0).start()

        @pl.when(layer == 0)
        def _():
            for c in wqkv_copies:
                c.start()
            rng_reset()

            def ln_first(t):
                r0 = pl.multiple_of(jnp.minimum(t, nt - 1) * TM, TM)
                return _layernorm(x_in[pl.ds(r0, TS), :].astype(F32)).astype(BF16)

            x_copy(0).wait()
            xns = []
            for r0 in range(0, TM, TS):
                xt = x_in[r0:r0 + TS, :].astype(F32)
                x[r0:r0 + TS, :] = xt
                xns.append((r0, _layernorm(xt).astype(BF16)))
            for c, mm in zip(wqkv_copies, (k_mm, q_mm, v_mm)):
                c.wait()
                if mm is k_mm:
                    x_copy(1).start()
                if mm is v_mm:
                    x_copy(1).wait()
                    for t in range(2, nt):
                        x_copy(t).start()
                for r0, xn in xns:
                    mm(r0, xn)
            xn0 = ln_first(1)
            for c in ffn_copies:
                c.start()

            def body(t, xn0, tables):
                @pl.when(t + 1 < nt)
                def _():
                    x_copy(t + 1).wait()

                if tables:
                    prep_tables(t)
                res = []
                for n, r0 in enumerate(subrows(t, TM)):
                    xt = x_in[pl.ds(r0, TS), :].astype(F32)
                    x[pl.ds(r0, TS), :] = xt
                    res += qkv_mm(r0, xn0 if n == 0 else _layernorm(xt).astype(BF16))
                if tables:
                    jobs = []
                    for w, ws, swap in ((w1, w1s, False), (w2, w2s, True)):
                        rb = w.shape[0] // nt
                        r0 = (t - nt // 2) * rb
                        jobs += [(w, ws, swap, pl.multiple_of(r0 + r, 16), c)
                                 for r in range(0, rb, 16)
                                 for c in range(0, w.shape[1] // 2, 128)]
                    for n, job in enumerate(jobs):
                        strassen_weights(*job, res[n * (len(res) * 5 // 6) // len(jobs)])
                return ln_first(t + 1)
            xn0 = lax.fori_loop(1, nt // 2, lambda t, c: body(t, c, False), xn0)
            for c in ffn_copies:
                c.wait()
            lax.fori_loop(nt // 2, nt, lambda t, c: body(t, c, True), xn0)
            for c in late_copies:
                c.start()

        attention()

        @pl.when(layer == 0)
        def _():
            for c in late_copies:
                c.wait()

            def body(t, o0):
                rl = subrows(t, TM)
                prep_tables(t)
                for r0, x2 in zip(rl, post_tiles(rl, o0)):
                    x[pl.ds(r0, TS), :] = x2
                    qkv_mm(r0, _layernorm(x2).astype(BF16))
                return o_first(t + 1, TM)
            lax.fori_loop(0, nt, body, pltpu.bitcast(o0buf[...], BF16))

        @pl.when(layer == 1)
        def _():
            def body(t, o0):
                rl = subrows(t, TM_LAST)
                for n, (r0, x2) in enumerate(zip(rl, post_tiles(rl, o0))):
                    out[pl.ds(r0, TS), :] = x2.astype(out.dtype)
                    out_copy(t * (TM_LAST // TS) + n).start()
                return o_first(t + 1, TM_LAST)
            lax.fori_loop(0, S // TM_LAST, body, pltpu.bitcast(o0buf[...], BF16))
            for t in range(S // TS):
                out_copy(t).wait()

    scratch = [
        pltpu.VMEM((S, D), BF16),
        pltpu.VMEM((D, 3 * D), BF16),
        pltpu.VMEM((D, D), BF16),
        pltpu.VMEM((D, F), BF16),
        pltpu.VMEM((F, D), BF16),
        pltpu.VMEM((S, D), BF16),
        pltpu.VMEM((S, D), F32),
        pltpu.VMEM((H, DH // 2, S), U32),
        pltpu.VMEM((H, DH, S), F32),
        pltpu.VMEM((nslab, S // 2, 128), U32),
        pltpu.VMEM((H, DH, S), F32),
        pltpu.VMEM((H, DH, S), F32),
        pltpu.VMEM((D, S), BF16),
        pltpu.VMEM((H, 8, S), F32),
        pltpu.VMEM((nq, S, TQ), F32),
        pltpu.VMEM((nq, S, TQ), F32),
        pltpu.VMEM((DH, ngrp * 128, 128), F32),
        pltpu.VMEM((DH, ngrp * 128, 128), F32),
        pltpu.VMEM((S // 2, 128), U32),
        pltpu.VMEM((S // 2, 128), U32),
        pltpu.VMEM((DH, S), F32),
        pltpu.VMEM((DH, S), F32),
        pltpu.VMEM((H, 4, DH, 128), F32),
        pltpu.VMEM((DH, ngrp0 * 128 + 8, 128), F32),
        pltpu.VMEM((4, DH, 128), F32),
        pltpu.VMEM((TS // 2, D), U32),
        pltpu.VMEM((7, D // 4, F // 2), U32),
        pltpu.VMEM((7, F // 4, D // 2), U32),
        pltpu.VMEM((4, 8, 128), F32),
        pltpu.VMEM((F,), BF16),
        pltpu.VMEM((D,), BF16),
        pltpu.SemaphoreType.DMA((nt,)),
        pltpu.SemaphoreType.DMA((4,)),
        pltpu.SemaphoreType.DMA((1,)),
    ]
    return kernel, scratch


@jax.jit
def pallas_interleave_layers__mha_block__dense_activation_gelu__prompt_kernel(
    A_x: jax.Array,
    A_wqkv: jax.Array,
    A_wo: jax.Array,
    B_x: jax.Array,
    B_w1: jax.Array,
    B_b1: jax.Array,
    B_w2: jax.Array,
    B_b2: jax.Array,
):
    B, S, D = A_x.shape
    F = B_w1.shape[1]
    assert B == 1
    x2d = A_x.reshape(S, D)

    hbm = pl.BlockSpec(memory_space=pl.ANY)
    kernel, scratch = _make_kernel(S, D, F)

    out = pl.pallas_call(
        kernel,
        grid=(2,),
        in_specs=[hbm] * 7,
        out_specs=hbm,
        out_shape=jax.ShapeDtypeStruct((S, D), A_x.dtype),
        scratch_shapes=scratch,
        compiler_params=pltpu.CompilerParams(
            dimension_semantics=("arbitrary",),
            vmem_limit_bytes=100 * 1024 * 1024,
        ),
    )(x2d, A_wqkv, A_wo, B_w1, B_b1, B_w2, B_b2)
    return out.reshape(B, S, D)
```

```python
import math

import jax
import jax.numpy as jnp
from jax import lax
import jax.experimental.pallas as pl
import jax.experimental.pallas.tpu as pltpu

F32 = jnp.float32
BF16 = jnp.bfloat16
U32 = jnp.uint32

N_HEADS = 32
LN_EPS = 1e-5
TQ = 512
CK = 128
TS = 128
TM = 256
TE = 128
GV = 21
GV0 = 19
L_LO = 2.0 ** -20
L_HI = 2.0 ** 57
V_HI = 2.0 ** 60


def _layernorm(x):
    m = jnp.mean(x, axis=-1, keepdims=True)
    xc = x - m
    v = jnp.mean(xc * xc, axis=-1, keepdims=True)
    return xc * lax.rsqrt(v + LN_EPS)


def _gelu_tanh(x):
    c = math.sqrt(2.0 / math.pi)
    return 0.5 * x * (1.0 + jnp.tanh(c * (x + 0.044715 * (x * x * x))))


def _dot(a, b, dims=(((1,), (0,)), ((), ()))):
    return lax.dot_general(a, b, dims, precision=lax.Precision.DEFAULT,
                           preferred_element_type=F32)


def _make_kernel(S, D, F):
    H = N_HEADS
    DH = D // H
    HPG = 128 // DH
    nslab = D // 128
    nq = S // TQ
    nck = S // CK
    nt = S // TM
    ntl = TQ // 128
    nsteps = nq * nck
    qscale = (DH ** -0.5) * math.log2(math.e)
    ngrp = (GV * 16 + 127) // 128
    ngrp0 = (GV0 * 16 + 127) // 128
    assert nt == 2 * nslab and ngrp * 128 <= nslab * TM and DH % nslab == 0
    assert TM == 2 * TS and ntl == 4 and H % 2 == 0

    def plan(g):
        nm = S // 16 - g
        segs = [(nm * (c + 1)) // nck - (nm * c) // nck for c in range(nck)]
        pieces = sorted([(i, t) for i in range(g) for t in range(ntl)],
                        key=lambda p: ((p[0] + 5 * p[1]) % g, p[1]))
        pos = {}
        for n, p in enumerate(pieces):
            pos.setdefault(int((n + 0.5) * 2 * nm / len(pieces)), []).append(p)
        return segs, pos

    tr_pos = {}
    for n in range(DH * ngrp):
        tr_pos.setdefault(n * nsteps // (DH * ngrp), []).append(n)

    def kernel(x_hbm, wqkv_hbm, wo_hbm, w1_hbm, b1_hbm, w2_hbm, b2_hbm, out_hbm,
               x_in, wqkv, wo, w1, w2, out,
               x, qt, qf, k, vt, ot, on, ls, p0, p1, kb0, kb1, kr0, kr1, qs0, qs1,
               kto, kbz, kt0, o0buf, w1s, w2s, rng, b1, b2, xsem, wsem, osem):
        layer = pl.program_id(0)

        def x_copy(t):
            return pltpu.make_async_copy(x_hbm.at[pl.ds(t * TM, TM), :],
                                         x_in.at[pl.ds(t * TM, TM), :], xsem.at[t])

        def out_copy(t):
            return pltpu.make_async_copy(out.at[pl.ds(t * TS, TS), :],
                                         out_hbm.at[pl.ds(t * TS, TS), :], osem.at[0])

        wqkv_copies = [pltpu.make_async_copy(wqkv_hbm.at[:, pl.ds(c * D, D)],
                                             wqkv.at[:, pl.ds(c * D, D)], wsem.at[1 + c])
                       for c in (1, 0, 2)]
        ffn_copies = [pltpu.make_async_copy(src, dst, wsem.at[0])
                      for src, dst in ((w1_hbm, w1), (w2_hbm, w2))]
        late_copies = [pltpu.make_async_copy(src, dst, wsem.at[0])
                       for src, dst in ((wo_hbm, wo), (b1_hbm, b1), (b2_hbm, b2))]

        def rng_reset():
            rng[0] = jnp.full((8, 128), L_HI, F32)
            rng[1] = jnp.full((8, 128), L_LO, F32)
            rng[2] = jnp.zeros((8, 128), F32)

        tt_dims = (((0,), (1,)), ((), ()))

        def k_mm(r0, xn):
            kf = _dot(xn, wqkv[:, D:2 * D])
            kk = pltpu.bitcast(kf.astype(BF16), U32)
            for g in range(nslab):
                k[g, pl.ds(pl.multiple_of(r0 // 2, TS // 2), TS // 2), :] = (
                    kk[:, g * 128:(g + 1) * 128])
            return [(kf, r, c) for c in range(0, D, 128) for r in range(0, TS, 8)]

        def q_mm(r0, xn):
            rows = pl.ds(r0, TS)
            q = _dot(wqkv[:, 0:D], xn, tt_dims) * qscale
            qt[:, :, rows] = pltpu.bitcast(q.astype(BF16), U32).reshape(H, DH // 2, TS)
            qf[:, :, rows] = q.reshape(H, DH, TS)
            return [(q, r, 0) for r in range(0, D, 8)]

        def v_mm(r0, xn):
            v = _dot(wqkv[:, 2 * D:3 * D], xn, tt_dims)
            vt[:, :, pl.ds(r0, TS)] = v.reshape(H, DH, TS)
            rng[2] = jnp.maximum(rng[2], jnp.max(jnp.abs(v).reshape(D // 8, 8, TS), axis=0))
            return [(v, r, 0) for r in range(0, D, 8)]

        def qkv_mm(r0, xn):
            return k_mm(r0, xn) + q_mm(r0, xn) + v_mm(r0, xn)

        def subrows(t):
            return [pl.multiple_of(t * TM + i * TS, TS) for i in range(TM // TS)]

        def k_rot(h, r0, nr):
            kc = k[h // HPG, pl.ds(r0, nr), :]
            return pltpu.roll(kc, (128 - (h % HPG) * DH) % 128, 1)

        def prep(h, n, kb, kr, qs, hist, lag, off):
            nr = (S // 2) // nsteps
            if (n + 1) * nr * 2 > 16 * GV:
                kr[pl.ds(n * nr, nr), :] = k_rot(h, n * nr, nr)
            if n % 4 == 1:
                cols = pl.ds((n // 4) * 128, 128)
                qs[:, cols] = qf[h, :, cols]
            for idx in tr_pos.get(n, []):
                gi, d = idx // DH, idx % DH
                nk = min(128, GV * 16 - gi * 128)
                row = jnp.broadcast_to(kto[h, gi, d:d + 1, :], (8, 128))
                if len(hist) >= lag:
                    never = lax.broadcasted_iota(jnp.int32, (8, 128), 1) < -1 - layer
                    row = jnp.where(never, hist[-lag], row)
                v = jnp.concatenate([row] * 16, axis=0).T
                kb[d, gi * 128:gi * 128 + nk, :] = v[:nk]
                hist.append(v[off:off + 8])

        def prep_tables(t):
            nd = DH // nslab
            sl = t % nslab
            for gi in range(ngrp0):
                kt = pltpu.bitcast(k[0, gi * 64:(gi + 1) * 64, :], BF16).astype(F32).T
                kt0[gi] = kt[0:DH]
            for gi in range(ngrp):
                kt = pltpu.bitcast(k[sl, gi * 64:(gi + 1) * 64, :], BF16).astype(F32).T
                kto[pl.ds(sl * HPG, HPG), gi] = kt.reshape(HPG, DH, 128)
            for gi in range(ngrp0):
                nk = min(128, GV0 * 16 - gi * 128)
                for e in range(nd):
                    d = sl * nd + e
                    row = kt0[gi, pl.ds(d, 1), :]
                    kbz[d, gi * 128:gi * 128 + nk, :] = (
                        jnp.broadcast_to(row, (128, 128)).T[:nk])

        def piece(p, kba, qs, pbuf, j, l):
            i, t = p
            c0 = j * TQ + t * 128
            accs = {}
            for d in range(DH):
                qb = jnp.broadcast_to(qs[d:d + 1, c0:c0 + 128], (8, 128))
                for r in range(2):
                    o = 16 * i + r * 8
                    pr = kba[d, o:o + 8, :] * qb
                    key = (r, d % 2)
                    accs[key] = accs[key] + pr if key in accs else pr
            for r in range(2):
                e = jnp.exp2(accs[r, 0] + accs[r, 1])
                l[t] = l[t] + e
                pbuf[j, pl.ds(16 * i + r * 8, 8), t * 128:(t + 1) * 128] = e

        def normalize(h, cols, o):
            lsum = jnp.sum(ls[h, :, cols], axis=0, keepdims=True)
            r0 = pl.reciprocal(lsum, approx=True)
            rinv = r0 * (2.0 - lsum * r0)
            on[h * DH:(h + 1) * DH, cols] = (o * rinv).astype(BF16)

        def step(ha, pa, kba, kra, qsa, hb, pb, hn, kbn, krn, qsn):
            gv = GV0 if hb is None else GV
            segs, pos = plan(gv)
            hist = []
            for j in range(nq):
                if ha is not None:
                    w = pltpu.bitcast(qt[ha, :, pl.ds(j * TQ, TQ)], BF16)
                acc = None
                l = [None] * ntl
                g0 = gv
                for c in range(nck):
                    if ha is not None:
                        nm = segs[c] * 16
                        kc = pltpu.bitcast(kra[pl.ds(g0 * 8, nm // 2), :], BF16)
                        p = jnp.exp2(_dot(kc[:, 0:DH], w))
                        pa[j, pl.ds(g0 * 16, nm), :] = p
                        for r in range(nm // 8):
                            for t in range(ntl):
                                pr = p[r * 8:(r + 1) * 8, t * 128:(t + 1) * 128]
                                l[t] = pr if l[t] is None else l[t] + pr
                            for pc in pos.get((g0 - gv) * 2 + r, []):
                                piece(pc, kba, qsa, pa, j, l)
                        g0 += segs[c]
                    if hb is not None:
                        o = _dot(vt[hb, :, pl.ds(c * CK, CK)], pb[j, pl.ds(c * CK, CK), :])
                        acc = o if acc is None else o + acc
                    if hn is not None:
                        prep(hn, j * nck + c, kbn, krn, qsn, hist,
                             *((2, 64) if hb is None else (1, 0)))
                    if ha is None:
                        n = j * nck + c
                        hd, part = n % H, n // H
                        cw = S * H // nsteps
                        if hd != hb:
                            cols = pl.ds(part * cw, cw)
                            normalize(hd, cols, ot[hd, :, cols])
                        if n == H + 8:
                            o0buf[...] = pltpu.bitcast(on[:, 0:TS].T, U32)
                if ha is None:
                    normalize(hb, pl.ds(j * TQ, TQ), acc)
                elif hb is not None:
                    ot[hb, :, pl.ds(j * TQ, TQ)] = acc
                if ha is not None:
                    ls[ha, :, pl.ds(j * TQ, TQ)] = jnp.concatenate(l, axis=1)
                    rng[0] = jnp.minimum(rng[0], jnp.minimum(jnp.minimum(l[0], l[1]),
                                                             jnp.minimum(l[2], l[3])))
                    rng[1] = jnp.maximum(rng[1], jnp.maximum(jnp.maximum(l[0], l[1]),
                                                             jnp.maximum(l[2], l[3])))

        def exact_attention():
            ne = S // TE

            def body(u, carry):
                h = u // ne
                cols = pl.ds(pl.multiple_of((u % ne) * TE, TE), TE)
                w = pltpu.bitcast(qt[h, :, cols], BF16)
                kc = pltpu.bitcast(k_rot(h, 0, S // 2), BF16)
                s = _dot(kc[:, 0:DH], w)
                p = jnp.exp2(s - jnp.max(s, axis=0, keepdims=True))
                o = _dot(vt[h], p) / jnp.sum(p, axis=0, keepdims=True)
                on[pl.ds(pl.multiple_of(h * DH, DH), DH), cols] = o.astype(BF16)
                return carry
            lax.fori_loop(0, H * ne, body, 0)
            o0buf[...] = pltpu.bitcast(on[:, 0:TS].T, U32)

        def attention():
            step(0, p0, kbz, k.at[0], qf.at[0], None, None, 1, kb1, kr1, qs1)

            def body(i, carry):
                h = 2 * i
                step(h + 1, p1, kb1, kr1, qs1, h, p0,
                     jnp.minimum(h + 2, H - 1), kb0, kr0, qs0)

                @pl.when(h + 2 < H)
                def _():
                    step(h + 2, p0, kb0, kr0, qs0, h + 1, p1, h + 3, kb1, kr1, qs1)
                return carry
            lax.fori_loop(0, H // 2, body, 0)
            ok = (rng[0] >= L_LO) & (rng[1] <= L_HI) & (rng[2] <= V_HI)
            nbad = jnp.max(jnp.where(ok, 0.0, 1.0))
            rng_reset()
            step(None, None, None, None, None, H - 1, p1, None, None, None, None)

            @pl.when(nbad > 0.0)
            def _():
                exact_attention()

        def strassen(a11, a12, a21, a22, ws):
            def mm(a, i):
                return _dot(a.astype(BF16), pltpu.bitcast(ws[i - 1], BF16))
            m3 = mm(a11, 3)
            m5 = mm(a11 + a12, 5)
            m2 = mm(a21 + a22, 2)
            m4 = mm(a22, 4)
            m1 = mm(a11 + a22, 1)
            m7 = mm(a12 - a22, 7)
            m6 = mm(a21 - a11, 6)
            return [m4 - m5 + m1 + m7, m3 + m5, m2 + m4, m3 - m2 + m1 + m6]

        def strassen_weights(w, ws, r0, c0, tie):
            kh, nh = w.shape[0] // 2, w.shape[1] // 2
            never = lax.broadcasted_iota(jnp.int32, (8, 128), 1) < -1 - layer
            tie = pltpu.bitcast(tie, U32)

            def blk(r, c):
                v = pltpu.bitcast(w[pl.ds(r + r0, 16), c + c0:c + c0 + 128], U32)
                return pltpu.bitcast(jnp.where(never, tie, v), BF16)
            b11, b12, b21, b22 = blk(0, 0), blk(0, nh), blk(kh, 0), blk(kh, nh)
            f11, f12, f21, f22 = [b.astype(F32) for b in (b11, b12, b21, b22)]
            rows = pl.ds(pl.multiple_of(r0 // 2, 8), 8)
            for n, v in enumerate((f11 + f22, b11, f12 - f22, f21 - f11, b22,
                                   f11 + f12, f21 + f22)):
                ws[n, rows, c0:c0 + 128] = pltpu.bitcast(v.astype(BF16), U32)

        def o_first(t):
            r0 = pl.multiple_of(jnp.minimum(t, nt - 1) * TM, TM)
            return on[:, pl.ds(r0, TS)].T

        def post_tiles(r0s, o0):
            x1s = []
            for n, r0 in enumerate(r0s):
                if n == 0:
                    attn = _dot(o0, wo[...])
                else:
                    attn = _dot(on[:, pl.ds(r0, TS)], wo[...], (((0,), (0,)), ((), ())))
                x1s.append(x[pl.ds(r0, TS), :] + attn)
            top, bot = [_layernorm(x1) for x1 in x1s]
            b1f = b1[...].astype(F32)
            b2f = b2[...].astype(F32)
            c = strassen(top[:, :D // 2], top[:, D // 2:], bot[:, :D // 2], bot[:, D // 2:], w1s)
            hid = [_gelu_tanh(ci + bi)
                   for ci, bi in zip(c, (b1f[:F // 2], b1f[F // 2:]) * 2)]
            c = strassen(*hid, w2s)
            return [x1s[0] + (jnp.concatenate(c[0:2], axis=1) + b2f),
                    x1s[1] + (jnp.concatenate(c[2:4], axis=1) + b2f)]

        @pl.when(layer < 1)
        def _():
            x_copy(0).start()

        @pl.when(layer == 0)
        def _():
            for c in wqkv_copies:
                c.start()
            rng_reset()

            def ln_first(t):
                r0 = pl.multiple_of(jnp.minimum(t, nt - 1) * TM, TM)
                return _layernorm(x_in[pl.ds(r0, TS), :].astype(F32)).astype(BF16)

            x_copy(0).wait()
            xns = []
            for r0 in range(0, TM, TS):
                xt = x_in[r0:r0 + TS, :].astype(F32)
                x[r0:r0 + TS, :] = xt
                xns.append((r0, _layernorm(xt).astype(BF16)))
            for c, mm in zip(wqkv_copies, (k_mm, q_mm, v_mm)):
                c.wait()
                if mm is k_mm:
                    x_copy(1).start()
                if mm is v_mm:
                    x_copy(1).wait()
                    for t in range(2, nt):
                        x_copy(t).start()
                for r0, xn in xns:
                    mm(r0, xn)
            xn0 = ln_first(1)
            for c in ffn_copies:
                c.start()

            def body(t, xn0, tables):
                @pl.when(t + 1 < nt)
                def _():
                    x_copy(t + 1).wait()

                if tables:
                    prep_tables(t)
                res = []
                for n, r0 in enumerate(subrows(t)):
                    xt = x_in[pl.ds(r0, TS), :].astype(F32)
                    x[pl.ds(r0, TS), :] = xt
                    res += qkv_mm(r0, xn0 if n == 0 else _layernorm(xt).astype(BF16))
                if tables:
                    jobs = []
                    for w, ws in ((w1, w1s), (w2, w2s)):
                        rb = w.shape[0] // nt
                        r0 = (t - nt // 2) * rb
                        jobs += [(w, ws, pl.multiple_of(r0 + r, 16), c)
                                 for r in range(0, rb, 16)
                                 for c in range(0, w.shape[1] // 2, 128)]
                    for n, job in enumerate(jobs):
                        a, r, c = res[n * (len(res) * 5 // 6) // len(jobs)]
                        strassen_weights(*job, a[r:r + 8, c:c + 128])
                return ln_first(t + 1)
            xn0 = lax.fori_loop(1, nt // 2, lambda t, c: body(t, c, False), xn0)
            for c in ffn_copies:
                c.wait()
            lax.fori_loop(nt // 2, nt, lambda t, c: body(t, c, True), xn0)
            for c in late_copies:
                c.start()

        attention()

        @pl.when(layer == 0)
        def _():
            for c in late_copies:
                c.wait()

            def body(t, o0):
                rl = subrows(t)
                prep_tables(t)
                for r0, x2 in zip(rl, post_tiles(rl, o0)):
                    x[pl.ds(r0, TS), :] = x2
                    qkv_mm(r0, _layernorm(x2).astype(BF16))
                return o_first(t + 1)
            lax.fori_loop(0, nt, body, pltpu.bitcast(o0buf[...], BF16))

        @pl.when(layer == 1)
        def _():
            def body(t, o0):
                rl = subrows(t)
                for n, (r0, x2) in enumerate(zip(rl, post_tiles(rl, o0))):
                    out[pl.ds(r0, TS), :] = x2.astype(out.dtype)
                    out_copy(t * (TM // TS) + n).start()
                return o_first(t + 1)
            lax.fori_loop(0, nt, body, pltpu.bitcast(o0buf[...], BF16))
            for t in range(S // TS):
                out_copy(t).wait()

    scratch = [
        pltpu.VMEM((S, D), BF16),
        pltpu.VMEM((D, 3 * D), BF16),
        pltpu.VMEM((D, D), BF16),
        pltpu.VMEM((D, F), BF16),
        pltpu.VMEM((F, D), BF16),
        pltpu.VMEM((S, D), BF16),
        pltpu.VMEM((S, D), F32),
        pltpu.VMEM((H, DH // 2, S), U32),
        pltpu.VMEM((H, DH, S), F32),
        pltpu.VMEM((nslab, S // 2, 128), U32),
        pltpu.VMEM((H, DH, S), F32),
        pltpu.VMEM((H, DH, S), F32),
        pltpu.VMEM((D, S), BF16),
        pltpu.VMEM((H, 8, S), F32),
        pltpu.VMEM((nq, S, TQ), F32),
        pltpu.VMEM((nq, S, TQ), F32),
        pltpu.VMEM((DH, ngrp * 128, 128), F32),
        pltpu.VMEM((DH, ngrp * 128, 128), F32),
        pltpu.VMEM((S // 2, 128), U32),
        pltpu.VMEM((S // 2, 128), U32),
        pltpu.VMEM((DH, S), F32),
        pltpu.VMEM((DH, S), F32),
        pltpu.VMEM((H, 4, DH, 128), F32),
        pltpu.VMEM((DH, ngrp0 * 128 + 8, 128), F32),
        pltpu.VMEM((4, DH, 128), F32),
        pltpu.VMEM((TS // 2, D), U32),
        pltpu.VMEM((7, D // 4, F // 2), U32),
        pltpu.VMEM((7, F // 4, D // 2), U32),
        pltpu.VMEM((4, 8, 128), F32),
        pltpu.VMEM((F,), BF16),
        pltpu.VMEM((D,), BF16),
        pltpu.SemaphoreType.DMA((nt,)),
        pltpu.SemaphoreType.DMA((4,)),
        pltpu.SemaphoreType.DMA((1,)),
    ]
    return kernel, scratch


@jax.jit
def pallas_interleave_layers__mha_block__dense_activation_gelu__prompt_kernel(
    A_x: jax.Array,
    A_wqkv: jax.Array,
    A_wo: jax.Array,
    B_x: jax.Array,
    B_w1: jax.Array,
    B_b1: jax.Array,
    B_w2: jax.Array,
    B_b2: jax.Array,
):
    B, S, D = A_x.shape
    F = B_w1.shape[1]
    assert B == 1
    x2d = A_x.reshape(S, D)

    hbm = pl.BlockSpec(memory_space=pl.ANY)
    kernel, scratch = _make_kernel(S, D, F)

    out = pl.pallas_call(
        kernel,
        grid=(2,),
        in_specs=[hbm] * 7,
        out_specs=hbm,
        out_shape=jax.ShapeDtypeStruct((S, D), A_x.dtype),
        scratch_shapes=scratch,
        compiler_params=pltpu.CompilerParams(
            dimension_semantics=("arbitrary",),
            vmem_limit_bytes=100 * 1024 * 1024,
        ),
    )(x2d, A_wqkv, A_wo, B_w1, B_b1, B_w2, B_b2)
    return out.reshape(B, S, D)
```
